```python
import os as _os
_os.environ.setdefault("JAX_PLATFORMS", "cpu")
import jax
import jax.numpy as jnp

def _softmax(x, axis=-1):
    return jax.nn.softmax(x, axis=axis)
def _gelu(x):
    return jax.nn.gelu(x, approximate=True)
def _silu(x):
    return jax.nn.silu(x)
def _sigmoid(x):
    return jax.nn.sigmoid(x)
def _layernorm(x, axis=-1, eps=1e-5):
    m = jnp.mean(x, axis=axis, keepdims=True)
    v = jnp.var(x, axis=axis, keepdims=True)
    return (x - m) / jnp.sqrt(v + eps)
def _scatter_add(tgt, idx, src, axis=0):
    return tgt.at[idx].add(src)
def _segment_sum(src, seg, n):
    return jax.ops.segment_sum(src, seg, n)
class _Rng:
    def __init__(self, key):
        self._k = key
    def _next(self):
        self._k, sub = jax.random.split(self._k)
        return sub
    def normal(self, shape):
        return jax.random.normal(self._next(), shape, dtype=jnp.bfloat16)
    def randint(self, lo, hi, shape):
        return jax.random.randint(self._next(), shape, lo, hi, dtype=jnp.int32)
    def uniform(self, shape, lo=0.0, hi=1.0):
        return jax.random.uniform(self._next(), shape, jnp.bfloat16, lo, hi)
    def permutation(self, n):
        return jax.random.permutation(self._next(), n)


kernel_name = 'gated_mix__mha_block__softmax_full_mha__prompt'

def setup_inputs():
    _rng = _Rng(jax.random.key(int.from_bytes(__import__("os").urandom(4), "little")))
    _w = (lambda a: (lambda t: t.astype(jnp.bfloat16) if jnp.issubdtype(t.dtype, jnp.floating) else t)(jnp.asarray(a)))
    def _A_setup():
        B, S, D, H = 1, 2048, 448, 16
        return {
            "x": _w((lambda *s: _rng.normal(s) * 0.05)(B, S, D)),
            "wqkv": _w((lambda *s: _rng.normal(s) * 0.4)(D, 3 * D)),
            "wo": _w((lambda *s: _rng.normal(s) * 0.05)(D, D)),
        }
    _A_in = _A_setup()

    def _B_setup():
        B, S, D = 1, 2048, 448
        return {
            "x": _w((lambda *s: _rng.normal(s) * 0.05)(B, S, D)),
            "wqkv": _w((lambda *s: _rng.normal(s) * 0.4)(D, 3 * D)),
            "wo": _w((lambda *s: _rng.normal(s) * 0.05)(D, D)),
        }
    _B_in = _B_setup()

    return {
        "A_x": _A_in["x"],
        "A_wqkv": _A_in["wqkv"],
        "A_wo": _A_in["wo"],
        "B_x": _B_in["x"],
        "B_wqkv": _B_in["wqkv"],
        "B_wo": _B_in["wo"],
        "gate_w": _w((lambda *s: _rng.normal(s) * 0.05)(448) * 16.0),
    }

def reference(A_x, A_wqkv, A_wo, B_x, B_wqkv, B_wo, gate_w):
    def _A_ref(x, wqkv, wo):
        B, S, D = x.shape
        H = 16
        Dh = D // H
        qkv = (lambda x, *d: x.transpose(*d))((x @ wqkv).reshape(B, S, 3, H, Dh), 2, 0, 3, 1, 4)
        q, k, v = qkv[0], qkv[1], qkv[2]
        scores = jnp.einsum("bhqd,bhkd->bhqk", q, k) * (Dh ** -0.5)
        p = _softmax(scores, axis=-1)
        o = jnp.einsum("bhqk,bhkd->bhqd", p, v)
        return (lambda x, *d: x.transpose(*d))(o, 0, 2, 1, 3).reshape(B, S, D) @ wo

    def _B_ref(x, wqkv, wo):
        B, S, D = x.shape
        H = 16; Dh = D // H
        qkv = (lambda x, *d: x.transpose(*d))((x @ wqkv).reshape(B, S, 3, H, Dh), 2, 0, 3, 1, 4)
        q, k, v = qkv[0], qkv[1], qkv[2]
        scale = Dh ** -0.5
        scores = jnp.einsum("bhqd,bhkd->bhqk", q, k) * scale
        p = _softmax(scores, axis=-1)
        o = jnp.einsum("bhqk,bhkd->bhqd", p, v)
        return (lambda x, *d: x.transpose(*d))(o, 0, 2, 1, 3).reshape(B, S, D) @ wo

    x = A_x
    g = _sigmoid((x * gate_w).sum(-1, keepdims=True))
    a = _A_ref(x, A_wqkv, A_wo)
    b = _B_ref(x, B_wqkv, B_wo)
    return g * a + (1 - g) * b
```

```python
import functools
import math

import jax
import jax.numpy as jnp
from jax import lax
import jax.experimental.pallas as pl
import jax.experimental.pallas.tpu as pltpu


_NT = (((1,), (1,)), ((), ()))
_NN = (((1,), (0,)), ((), ()))
_TN = (((0,), (0,)), ((), ()))
_F32 = jnp.float32
_BF16 = jnp.bfloat16

_H = 16
_HP = 32
_BQ = 512
_BK = 128
_SKIP = 0
_ORDER = 1
_MODE = 1
_FLAGS = None
_UNROLL = 2


def _sel(tp, a, dh, width):
    r = lax.broadcasted_iota(jnp.int32, (128, width), 0)
    s = lax.broadcasted_iota(jnp.int32, (128, width), 1)
    d = r & (_HP - 1)
    hit = (d < dh) & ((128 * a + s) == (4 * dh * tp + dh * (r >> 5) + d))
    return jnp.where(hit, 1.0, 0.0).astype(_BF16)


def _src_tiles(tp, dh):
    lo = 4 * dh * tp
    return sorted({lo // 128, (lo + 4 * dh - 1) // 128})


def _kernel(x_ref, wa_ref, woa_ref, wb_ref, wob_ref, gw_ref, o_ref,
            qt_s, k_s, vt_s, s0, s1, ot_s, wt_s, wk_s, wo_s, m_s, g_s, *, S, D):
    dh = D // _H
    ntile = _H // 4
    DP = ntile * 128
    nq = S // _BQ
    nch = S // _BK
    NU = 2 * _H
    qscale = (dh ** -0.5) * math.log2(math.e)
    i = pl.program_id(0)
    row = lax.broadcasted_iota(jnp.int32, (128, _BQ), 0)

    def getq(u, qb):
        qt = qt_s[u >> 2, :, pl.ds(pl.multiple_of(qb * _BQ, _BQ), _BQ)]
        return jnp.where((row >> 5) == (u & 3), qt, jnp.zeros_like(qt))

    def stage_a(u, qm, c, sbuf, mx):
        st = lax.dot_general(k_s[u >> 2, pl.ds(c * _BK, _BK), :], qm, _NN,
                             preferred_element_type=_F32)
        sbuf[pl.ds(c * _BK, _BK), :] = st
        cm = jnp.max(st.reshape(_BK // 8, 8, _BQ), axis=0)
        return cm if mx is None else jnp.maximum(mx, cm)

    def stage_b(u, c, sbuf, m, acc):
        p = jnp.exp2(sbuf[pl.ds(c * _BK, _BK), :] - m).astype(_BF16)
        vt = vt_s[u >> 2, pl.ds(pl.multiple_of((u & 3) * _HP, _HP), _HP), pl.ds(c * _BK, _BK)]
        r = lax.dot_general(vt, p, _NN, preferred_element_type=_F32)
        return r if acc is None else acc + r

    def finish(u, acc):
        gate = g_s[u >> 4, :, pl.ds(pl.multiple_of(i * _BQ, _BQ), _BQ)]
        o = acc * (gate / acc[dh:dh + 1, :])
        ot_s[pl.ds(pl.multiple_of(u * _HP, _HP), _HP), :] = o.astype(_BF16)

    @pl.when(i == 0)
    def _prologue():
        for b, (w_ref, wo_ref) in enumerate(((wa_ref, woa_ref), (wb_ref, wob_ref))):
            for t in range(ntile):
                for part in range(3):
                    tp = part * ntile + t
                    acc = None
                    for a in _src_tiles(tp, dh):
                        wd = min(128, 3 * D - 128 * a)
                        e = _sel(tp, a, dh, wd)
                        w = w_ref[:, 128 * a:128 * a + wd]
                        if part == 1:
                            r = lax.dot_general(w, e, _NT, preferred_element_type=_F32)
                        else:
                            r = lax.dot_general(e, w, _NT, preferred_element_type=_F32)
                        acc = r if acc is None else acc + r
                    if part == 1:
                        wk_s[b, :, 128 * t:128 * (t + 1)] = acc.astype(_BF16)
                    else:
                        r0 = (part // 2) * DP + 128 * t
                        wt_s[b, r0:r0 + 128, :] = acc.astype(_BF16)
                acc = None
                for a in _src_tiles(t, dh):
                    wd = min(128, D - 128 * a)
                    r = lax.dot_general(_sel(t, a, dh, wd), wo_ref[128 * a:128 * a + wd, :], _NN,
                                        preferred_element_type=_F32)
                    acc = r if acc is None else acc + r
                wo_s[:, b * DP + 128 * t:b * DP + 128 * (t + 1)] = acc.T.astype(_BF16)

        gw = jnp.broadcast_to(gw_ref[...], (16, D))
        is_one = (lax.broadcasted_iota(jnp.int32, (128, _BQ), 0) & (_HP - 1)) == dh

        def proj(c, carry):
            c0 = pl.multiple_of(c * _BQ, _BQ)
            xt = x_ref[:, pl.ds(c0, _BQ)]
            xc = xt.T
            logit = lax.dot_general(gw, xt, _NN, preferred_element_type=_F32)[0:1, :]
            g = jax.nn.sigmoid(logit)
            g_s[0, :, pl.ds(c0, _BQ)] = g
            g_s[1, :, pl.ds(c0, _BQ)] = 1.0 - g
            for b in range(2):
                kk = lax.dot_general(xc, wk_s[b], _NN, preferred_element_type=_F32)
                for t in range(ntile):
                    k_s[b * ntile + t, pl.ds(c0, _BQ), :] = kk[:, 128 * t:128 * (t + 1)].astype(_BF16)
                for t in range(ntile):
                    qt = lax.dot_general(wt_s[b, 128 * t:128 * (t + 1), :], xt, _NN,
                                         preferred_element_type=_F32)
                    qt_s[b * ntile + t, :, pl.ds(c0, _BQ)] = (qt * qscale).astype(_BF16)
                    vt = lax.dot_general(wt_s[b, DP + 128 * t:DP + 128 * (t + 1), :], xt, _NN,
                                         preferred_element_type=_F32)
                    vt_s[b * ntile + t, :, pl.ds(c0, _BQ)] = jnp.where(is_one, 1.0, vt).astype(_BF16)
            return carry

        lax.fori_loop(0, nq, proj, 0)

        qm = getq(0, 0)
        mx = None
        for c in range(nch):
            mx = stage_a(0, qm, c, s0, mx)
        m_s[...] = mx

    def step(u, m, sb, sa):
        un = u + 1
        last = un == NU
        qb = jnp.where(last, jnp.minimum(i + 1, nq - 1), i)
        un = jnp.where(last, 0, un)
        qm = getq(un, qb)
        mx = None
        acc = None
        m = jnp.max(m, axis=0, keepdims=True)
        seq = []
        lead = {0: 1, 1: 0, 2: 1, 3: 2, 4: 2}[_ORDER]
        for c in range(nch + lead):
            if c >= lead and lead == 0:
                seq.append(('b', c - lead))
            if c < nch:
                seq.append(('a', c))
            if c >= lead and lead > 0:
                seq.append(('b', c - lead))
        if _ORDER in (2, 4):
            seq.remove(('a', nch - 1))
            seq.append(('a', nch - 1))
        for kind, c in seq:
            if kind == 'a':
                mx = stage_a(un, qm, c, sa, mx)
            else:
                acc = stage_b(u, c, sb, m, acc)
                if c == nch - 1:
                    finish(u, acc)
        return mx

    def body(t, m):
        for r in range(0, _UNROLL, 2):
            m = step(_UNROLL * t + r, m, s0, s1)
            m = step(_UNROLL * t + r + 1, m, s1, s0)
        return m

    def body1(u, carry):
        @pl.when((u & 1) == 0)
        def _():
            m_s[...] = step(u, m_s[...], s0, s1)

        @pl.when((u & 1) == 1)
        def _():
            m_s[...] = step(u, m_s[...], s1, s0)
        return carry

    if not _SKIP:
        if _MODE == 0:
            m_s[...] = lax.fori_loop(0, NU // _UNROLL, body, m_s[...])
        else:
            lax.fori_loop(0, NU, body1, 0)

    out = lax.dot_general(wo_s[...], ot_s[...], _NN, preferred_element_type=_F32)
    o_ref[...] = out.astype(o_ref.dtype)


@jax.jit
def pallas_gated_mix__mha_block__softmax_full_mha__prompt_kernel(
    A_x: jax.Array,
    A_wqkv: jax.Array,
    A_wo: jax.Array,
    B_x: jax.Array,
    B_wqkv: jax.Array,
    B_wo: jax.Array,
    gate_w: jax.Array,
):
    del B_x
    B, S, D = A_x.shape
    assert B == 1 and D % _H == 0 and D // _H < _HP and S % _BQ == 0
    ng = 2 * _H // 4
    DP = (_H // 4) * 128

    def full(shape):
        return pl.BlockSpec(shape, lambda i: (0,) * len(shape))

    out = pl.pallas_call(
        functools.partial(_kernel, S=S, D=D),
        grid=(S // _BQ,),
        in_specs=[full((D, S)), full((D, 3 * D)), full((D, D)), full((D, 3 * D)), full((D, D)),
                  full((1, D))],
        out_specs=pl.BlockSpec((D, _BQ), lambda i: (0, i)),
        out_shape=jax.ShapeDtypeStruct((D, S), A_x.dtype),
        scratch_shapes=[
            pltpu.VMEM((ng, 128, S), _BF16),
            pltpu.VMEM((ng, S, 128), _BF16),
            pltpu.VMEM((ng, 128, S), _BF16),
            pltpu.VMEM((S, _BQ), _F32),
            pltpu.VMEM((S, _BQ), _F32),
            pltpu.VMEM((2 * DP, _BQ), _BF16),
            pltpu.VMEM((2, 2 * DP, D), _BF16),
            pltpu.VMEM((2, D, DP), _BF16),
            pltpu.VMEM((D, 2 * DP), _BF16),
            pltpu.VMEM((8, _BQ), _F32),
            pltpu.VMEM((2, 1, S), _F32),
        ],
        compiler_params=pltpu.CompilerParams(
            dimension_semantics=("arbitrary",),
            vmem_limit_bytes=100 * 1024 * 1024,
            **({} if _FLAGS is None else dict(flags=_FLAGS)),
        ),
    )(A_x.reshape(S, D).T, A_wqkv, A_wo, B_wqkv, B_wo, gate_w.reshape(1, D))
    return out.T.reshape(B, S, D)
```

```python
import functools
import math

import jax
import jax.numpy as jnp
from jax import lax
import jax.experimental.pallas as pl
import jax.experimental.pallas.tpu as pltpu


_NN = (((1,), (0,)), ((), ()))
_F32 = jnp.float32
_BF16 = jnp.bfloat16

_H = 16
_HP = 32
_BQ = 512
_BK = 128
_UNROLL = 8
_LEAD = 2


def _kernel(x_hbm, wa_hbm, woa_hbm, wb_hbm, wob_hbm, gw_ref, o_ref,
            qt_s, k_s, vt_s, s0, s1, ot_s, wta_s, wtb_s, wo_s, m_s, g_s, x_ref, w_s, wor_s, sems, *, S, D):
    dh = D // _H
    ntile = _H // 4
    nq = S // _BQ
    nch = S // _BK
    NU = 2 * _H
    qscale = (dh ** -0.5) * math.log2(math.e)
    i = pl.program_id(0)

    def getq(u, qb, j):
        cols = pl.ds(pl.multiple_of(qb * _BQ, _BQ), _BQ)
        parts = [jnp.zeros((_HP * j, _BQ), _BF16)] if j > 0 else []
        parts.append(qt_s[u >> 2, _HP * j:_HP * (j + 1), cols])
        if j < 3:
            parts.append(jnp.zeros((128 - _HP * (j + 1), _BQ), _BF16))
        return jnp.concatenate(parts, axis=0)

    def stage_a(u, qm, c, sbuf, mx):
        st = lax.dot_general(k_s[u >> 2, pl.ds(c * _BK, _BK), :], qm, _NN,
                             preferred_element_type=_F32)
        sbuf[pl.ds(c * _BK, _BK), :] = st
        cm = jnp.max(st.reshape(_BK // 8, 8, _BQ), axis=0)
        return cm if mx is None else jnp.maximum(mx, cm)

    def stage_b(u, j, c, sbuf, m, acc):
        p = jnp.exp2(sbuf[pl.ds(c * _BK, _BK), :] - m).astype(_BF16)
        vt = vt_s[u >> 2, _HP * j:_HP * (j + 1), pl.ds(c * _BK, _BK)]
        r = lax.dot_general(vt, p, _NN, preferred_element_type=_F32)
        return r if acc is None else acc + r

    def finish(u, j, acc):
        gate = g_s[u >> 4, :, pl.ds(pl.multiple_of(i * _BQ, _BQ), _BQ)]
        o = acc * (gate / acc[dh:dh + 1, :])
        sh = (dh * j) % 8
        assert sh in (0, 4)
        base = pl.multiple_of(u * dh - sh, 8)
        if sh:
            o = pltpu.roll(o, sh, 0)
            keep = lax.broadcasted_iota(jnp.int32, (8, _BQ), 0) < sh
            head = jnp.where(keep, ot_s[pl.ds(base, 8), :], o[0:8])
            o = jnp.concatenate([head, o[8:]], axis=0)
        ot_s[pl.ds(base, _HP), :] = o

    @pl.when(i == 0)
    def _prologue():
        rparts = [(r, min(r + 128, D)) for r in range(0, D, 128)]
        srcs = [(wa_hbm.at[r0:r1], w_s.at[0, r0:r1]) for r0, r1 in rparts]
        srcs += [(x_hbm.at[:, 0:_BQ], x_ref.at[:, 0:_BQ]), (x_hbm.at[:, _BQ:S], x_ref.at[:, _BQ:S]),
                 (wb_hbm, w_s.at[1]), (woa_hbm, wor_s.at[0:D]), (wob_hbm, wor_s.at[D:2 * D])]
        cps = [pltpu.make_async_copy(src, dst, sems.at[n]) for n, (src, dst) in enumerate(srcs)]
        cp_x0, cp_mid, cp_wo = cps[len(rparts)], cps[len(rparts) + 1:-2], cps[-2:]
        for cp in cps[:len(rparts) + 1]:
            cp.start()
        for n, (r0, r1) in enumerate(rparts):
            cps[n].wait()
            if n == len(rparts) - 1:
                for cp in cp_mid + cp_wo:
                    cp.start()
            wta_s[:, r0:r1] = w_s[0, r0:r1, :].T
        cp_x0.wait()
        WP = 512
        WE = (3 * D) // 128 * 128
        assert nq >= 4 and 2 * WP <= WE <= 3 * WP

        gw = jnp.broadcast_to(gw_ref[...].reshape(1, D), (16, D))
        prow = lax.broadcasted_iota(jnp.int32, (128, _BQ), 0) & (_HP - 1)

        def heads4(r, rr, t):
            parts = []
            for h in range(4 * t, 4 * t + 4):
                off = dh * h
                sh = off % 8
                assert sh in (0, 4)
                parts.append(r[off:off + _HP] if sh == 0 else rr[off - 4:off - 4 + _HP])
            return jnp.concatenate(parts, axis=0)

        def proj(c, carry, b):
            if b == 0:
                @pl.when(c == 1)
                def _():
                    for cp in cp_mid:
                        cp.wait()
                p0 = pl.multiple_of(jnp.clip((c - 1) * WP, 0, WE - WP), 128)
                bsrc = jnp.minimum(c, 1)
                wtb_s[pl.ds(p0, WP), :] = w_s[bsrc, :, pl.ds(p0, WP)].T
                wtb_s[WE:3 * D, :] = w_s[bsrc, :, WE:3 * D].T
            else:
                for tt in range(2):
                    r0 = pl.multiple_of(jnp.minimum(2 * c + tt, 2 * D // 128 - 1) * 128, 128)
                    wo_s[:, pl.ds(r0, 128)] = wor_s[pl.ds(r0, 128), :].T
            c0 = pl.multiple_of(c * _BQ, _BQ)
            cols = pl.ds(c0, _BQ)
            xt = x_ref[:, cols]
            if b == 0:
                logit = lax.dot_general(gw, xt, _NN, preferred_element_type=_F32)[0:1, :]
                g = jax.nn.sigmoid(logit)
                g_s[0, :, cols] = g
                g_s[1, :, cols] = 1.0 - g
            for part in range(3):
                r = lax.dot_general((wta_s, wtb_s)[b][part * D:(part + 1) * D, :], xt, _NN,
                                    preferred_element_type=_F32)
                rr = pltpu.roll(r, D - 4, 0)
                for t in range(ntile):
                    y = heads4(r, rr, t)
                    gi = b * ntile + t
                    if part == 0:
                        qt_s[gi, :, cols] = jnp.where(prow < dh, y * qscale, 0.0).astype(_BF16)
                    elif part == 1:
                        k_s[gi, cols, :] = jnp.where(prow < dh, y, 0.0).astype(_BF16).T
                    else:
                        y = jnp.where(prow < dh, y, jnp.where(prow == dh, 1.0, 0.0))
                        vt_s[gi, :, cols] = y.astype(_BF16)
            return carry

        lax.fori_loop(0, nq, functools.partial(proj, b=0), 0)
        for cp in cp_wo:
            cp.wait()
        lax.fori_loop(0, nq, functools.partial(proj, b=1), 0)

        qm = getq(0, 0, 0)
        mx = None
        for c in range(nch):
            mx = stage_a(0, qm, c, s0, mx)
        m_s[...] = mx

    def step(u, j, m, sb, sa, skip_a):
        un = u + 1
        last = un == NU
        qb = jnp.where(last, jnp.minimum(i + 1, nq - 1), i)
        un = jnp.where(last, 0, un)
        qm = getq(un, qb, (j + 1) % 4)
        m = jnp.broadcast_to(jnp.max(m, axis=0, keepdims=True), (8, _BQ))
        always = jnp.broadcast_to(g_s[0, :, 0:_BQ], (8, _BQ)) > -1.0
        mx, acc, toks = None, None, {}
        for n in range(nch + _LEAD):
            if n < nch and not skip_a:
                mx = stage_a(un, qm, n, sa, mx)
                toks[n] = mx
            c = n - _LEAD
            if c >= 0:
                mm = jnp.where(always, m, toks[c - _LEAD]) if (c - _LEAD) in toks else m
                acc = stage_b(u, j, c, sb, mm[0:1, :], acc)
        finish(u, j, acc)
        return m if skip_a else mx

    def region(t, final):
        m = m_s[...]
        for r in range(_UNROLL):
            j = r % 4
            sb, sa = (s0, s1) if j % 2 == 0 else (s1, s0)
            m = step(_UNROLL * t + r, j, m, sb, sa, skip_a=final and r == _UNROLL - 1)
        m_s[...] = m

    def body(t, carry):
        fin = jnp.logical_and(i == nq - 1, t == NU // _UNROLL - 1)
        pl.when(jnp.logical_not(fin))(functools.partial(region, t, False))
        pl.when(fin)(functools.partial(region, t, True))
        return carry

    lax.fori_loop(0, NU // _UNROLL, body, 0)

    out = lax.dot_general(wo_s[...], ot_s[...].astype(_BF16), _NN, preferred_element_type=_F32)
    o_ref[...] = out.astype(o_ref.dtype)


@jax.jit
def pallas_gated_mix__mha_block__softmax_full_mha__prompt_kernel(
    A_x: jax.Array,
    A_wqkv: jax.Array,
    A_wo: jax.Array,
    B_x: jax.Array,
    B_wqkv: jax.Array,
    B_wo: jax.Array,
    gate_w: jax.Array,
):
    del B_x
    B, S, D = A_x.shape
    assert B == 1 and D % _H == 0 and D // _H < _HP and S == 4 * _BQ and (2 * D) % 128 == 0
    ng = 2 * _H // 4

    def full(shape):
        return pl.BlockSpec(shape, lambda i: (0,) * len(shape))

    out = pl.pallas_call(
        functools.partial(_kernel, S=S, D=D),
        grid=(S // _BQ,),
        in_specs=[pl.BlockSpec(memory_space=pl.ANY)] * 5 + [full((D,))],
        out_specs=pl.BlockSpec((D, _BQ), lambda i: (0, i)),
        out_shape=jax.ShapeDtypeStruct((D, S), A_x.dtype),
        scratch_shapes=[
            pltpu.VMEM((ng, 128, S), _BF16),
            pltpu.VMEM((ng, S, 128), _BF16),
            pltpu.VMEM((ng, 128, S), _BF16),
            pltpu.VMEM((S, _BQ), _F32),
            pltpu.VMEM((S, _BQ), _F32),
            pltpu.VMEM((2 * D, _BQ), _F32),
            pltpu.VMEM((3 * D, D), _BF16),
            pltpu.VMEM((3 * D, D), _BF16),
            pltpu.VMEM((D, 2 * D), _BF16),
            pltpu.VMEM((8, _BQ), _F32),
            pltpu.VMEM((2, 1, S), _F32),
            pltpu.VMEM((D, S), _BF16),
            pltpu.VMEM((2, D, 3 * D), _BF16),
            pltpu.VMEM((2 * D, D), _BF16),
            pltpu.SemaphoreType.DMA((9,)),
        ],
        compiler_params=pltpu.CompilerParams(
            dimension_semantics=("arbitrary",),
            vmem_limit_bytes=100 * 1024 * 1024,
        ),
    )(A_x.reshape(S, D).T, A_wqkv, A_wo, B_wqkv, B_wo, gate_w)
    return out.T.reshape(B, S, D)
```

```python
import functools
import math

import jax
import jax.numpy as jnp
from jax import lax
import jax.experimental.pallas as pl
import jax.experimental.pallas.tpu as pltpu


_NN = (((1,), (0,)), ((), ()))
_F32 = jnp.float32
_BF16 = jnp.bfloat16

_H = 16
_HP = 32
_BQ = 512
_BK = 128
_UNROLL = 8
_LEAD = 2


def _kernel(x_hbm, wa_hbm, woa_hbm, wb_hbm, wob_hbm, gw_ref, o_ref,
            qt_s, k_s, vt_s, s0, s1, ot_s, wta_s, wtb_s, wo_s, m_s, g_s, x_ref, w_s, wor_s, sems, *, S, D):
    dh = D // _H
    ntile = _H // 4
    nq = S // _BQ
    nch = S // _BK
    NU = 2 * _H
    qscale = (dh ** -0.5) * math.log2(math.e)
    i = pl.program_id(0)

    def getq(u, qb, j):
        cols = pl.ds(pl.multiple_of(qb * _BQ, _BQ), _BQ)
        parts = [jnp.zeros((_HP * j, _BQ), _BF16)] if j > 0 else []
        parts.append(qt_s[u >> 2, _HP * j:_HP * (j + 1), cols])
        if j < 3:
            parts.append(jnp.zeros((128 - _HP * (j + 1), _BQ), _BF16))
        return jnp.concatenate(parts, axis=0)

    def stage_a(u, qm, c, sbuf, mx):
        st = lax.dot_general(k_s[u >> 2, pl.ds(c * _BK, _BK), :], qm, _NN,
                             preferred_element_type=_F32)
        sbuf[pl.ds(c * _BK, _BK), :] = st
        cm = jnp.max(st.reshape(_BK // 8, 8, _BQ), axis=0)
        return cm if mx is None else jnp.maximum(mx, cm)

    def stage_b(u, j, c, sbuf, m, acc):
        p = jnp.exp2(sbuf[pl.ds(c * _BK, _BK), :] - m).astype(_BF16)
        vt = vt_s[u >> 2, _HP * j:_HP * (j + 1), pl.ds(c * _BK, _BK)]
        r = lax.dot_general(vt, p, _NN, preferred_element_type=_F32)
        return r if acc is None else acc + r

    def finish(u, j, acc):
        gate = g_s[u >> 4, :, pl.ds(pl.multiple_of(i * _BQ, _BQ), _BQ)]
        o = acc * (gate / acc[dh:dh + 1, :])
        sh = (dh * j) % 8
        assert sh in (0, 4)
        base = pl.multiple_of(u * dh - sh, 8)
        if sh:
            o = pltpu.roll(o, sh, 0)
            keep = lax.broadcasted_iota(jnp.int32, (8, _BQ), 0) < sh
            head = jnp.where(keep, ot_s[pl.ds(base, 8), :], o[0:8])
            o = jnp.concatenate([head, o[8:]], axis=0)
        ot_s[pl.ds(base, _HP), :] = o

    @pl.when(i == 0)
    def _prologue():
        rparts = [(r, min(r + 128, D)) for r in range(0, D, 128)]
        srcs = [(wa_hbm.at[r0:r1], w_s.at[0, r0:r1]) for r0, r1 in rparts]
        srcs += [(x_hbm.at[:, _BQ * n:_BQ * (n + 1)], x_ref.at[:, _BQ * n:_BQ * (n + 1)]) for n in range(nq)]
        srcs += [(wb_hbm, w_s.at[1]), (woa_hbm, wor_s.at[0:D]), (wob_hbm, wor_s.at[D:2 * D])]
        cps = [pltpu.make_async_copy(src, dst, sems.at[n]) for n, (src, dst) in enumerate(srcs)]
        cp_x, cp_wb, cp_wo = cps[len(rparts):len(rparts) + nq], cps[-3], cps[-2:]
        for cp in cps[:len(rparts) + 1]:
            cp.start()
        for n, (r0, r1) in enumerate(rparts):
            cps[n].wait()
            if n == len(rparts) - 1:
                cp_x[1].start()
                cp_wb.start()
            wta_s[:, r0:r1] = w_s[0, r0:r1, :].T
        cp_x[0].wait()
        WP = 512
        WE = (3 * D) // 128 * 128
        assert nq == 4 and 2 * WP <= WE <= 3 * WP

        gw = jnp.broadcast_to(gw_ref[...].reshape(1, D), (16, D))
        prow = lax.broadcasted_iota(jnp.int32, (128, _BQ), 0) & (_HP - 1)

        def heads4(r, rr, t):
            parts = []
            for h in range(4 * t, 4 * t + 4):
                off = dh * h
                sh = off % 8
                assert sh in (0, 4)
                parts.append(r[off:off + _HP] if sh == 0 else rr[off - 4:off - 4 + _HP])
            return jnp.concatenate(parts, axis=0)

        def proj(c, carry, b):
            if b == 0:
                @pl.when(c == 1)
                def _():
                    cp_x[1].wait()
                    cp_wb.wait()
                    cp_x[2].start()
                    cp_x[3].start()

                @pl.when(c == 2)
                def _():
                    cp_x[2].wait()
                    for cp in cp_wo:
                        cp.start()

                @pl.when(c == 3)
                def _():
                    cp_x[3].wait()

                p0 = pl.multiple_of(jnp.clip((c - 1) * WP, 0, WE - WP), 128)
                bsrc = jnp.minimum(c, 1)
                wtb_s[pl.ds(p0, WP), :] = w_s[bsrc, :, pl.ds(p0, WP)].T
                wtb_s[WE:3 * D, :] = w_s[bsrc, :, WE:3 * D].T
            else:
                for tt in range(2):
                    r0 = pl.multiple_of(jnp.minimum(2 * c + tt, 2 * D // 128 - 1) * 128, 128)
                    wo_s[:, pl.ds(r0, 128)] = wor_s[pl.ds(r0, 128), :].T
            c0 = pl.multiple_of(c * _BQ, _BQ)
            cols = pl.ds(c0, _BQ)
            xt = x_ref[:, cols]
            if b == 0:
                logit = lax.dot_general(gw, xt, _NN, preferred_element_type=_F32)[0:1, :]
                g = jax.nn.sigmoid(logit)
                g_s[0, :, cols] = g
                g_s[1, :, cols] = 1.0 - g
            for part in range(3):
                r = lax.dot_general((wta_s, wtb_s)[b][part * D:(part + 1) * D, :], xt, _NN,
                                    preferred_element_type=_F32)
                rr = pltpu.roll(r, D - 4, 0)
                for t in range(ntile):
                    y = heads4(r, rr, t)
                    gi = b * ntile + t
                    if part == 0:
                        qt_s[gi, :, cols] = jnp.where(prow < dh, y * qscale, 0.0).astype(_BF16)
                    elif part == 1:
                        k_s[gi, cols, :] = jnp.where(prow < dh, y, 0.0).astype(_BF16).T
                    else:
                        y = jnp.where(prow < dh, y, jnp.where(prow == dh, 1.0, 0.0))
                        vt_s[gi, :, cols] = y.astype(_BF16)
            return carry

        lax.fori_loop(0, nq, functools.partial(proj, b=0), 0)
        for cp in cp_wo:
            cp.wait()
        lax.fori_loop(0, nq, functools.partial(proj, b=1), 0, unroll=2)

        qm = getq(0, 0, 0)
        mx = None
        for c in range(nch):
            mx = stage_a(0, qm, c, s0, mx)
        m_s[...] = mx

    def step(u, j, m, sb, sa, skip_a):
        un = u + 1
        last = un == NU
        qb = jnp.where(last, jnp.minimum(i + 1, nq - 1), i)
        un = jnp.where(last, 0, un)
        qm = getq(un, qb, (j + 1) % 4)
        m = jnp.broadcast_to(jnp.max(m, axis=0, keepdims=True), (8, _BQ))
        always = jnp.broadcast_to(g_s[0, :, 0:_BQ], (8, _BQ)) > -1.0
        mx, acc, toks = None, None, {}
        for n in range(nch + _LEAD):
            if n < nch and not skip_a:
                mx = stage_a(un, qm, n, sa, mx)
                toks[n] = mx
            c = n - _LEAD
            if c >= 0:
                mm = jnp.where(always, m, toks[c - _LEAD]) if (c - _LEAD) in toks else m
                acc = stage_b(u, j, c, sb, mm[0:1, :], acc)
        finish(u, j, acc)
        return m if skip_a else mx

    def region(t, final):
        m = m_s[...]
        for r in range(_UNROLL):
            j = r % 4
            sb, sa = (s0, s1) if j % 2 == 0 else (s1, s0)
            m = step(_UNROLL * t + r, j, m, sb, sa, skip_a=final and r == _UNROLL - 1)
        m_s[...] = m

    def body(t, carry):
        fin = jnp.logical_and(i == nq - 1, t == NU // _UNROLL - 1)
        pl.when(jnp.logical_not(fin))(functools.partial(region, t, False))
        pl.when(fin)(functools.partial(region, t, True))
        return carry

    lax.fori_loop(0, NU // _UNROLL, body, 0)

    out = lax.dot_general(wo_s[...], ot_s[...].astype(_BF16), _NN, preferred_element_type=_F32)
    o_ref[...] = out.astype(o_ref.dtype)


@jax.jit
def pallas_gated_mix__mha_block__softmax_full_mha__prompt_kernel(
    A_x: jax.Array,
    A_wqkv: jax.Array,
    A_wo: jax.Array,
    B_x: jax.Array,
    B_wqkv: jax.Array,
    B_wo: jax.Array,
    gate_w: jax.Array,
):
    del B_x
    B, S, D = A_x.shape
    assert B == 1 and D % _H == 0 and D // _H < _HP and S == 4 * _BQ and (2 * D) % 128 == 0
    ng = 2 * _H // 4

    def full(shape):
        return pl.BlockSpec(shape, lambda i: (0,) * len(shape))

    out = pl.pallas_call(
        functools.partial(_kernel, S=S, D=D),
        grid=(S // _BQ,),
        in_specs=[pl.BlockSpec(memory_space=pl.ANY)] * 5 + [full((D,))],
        out_specs=pl.BlockSpec((D, _BQ), lambda i: (0, i)),
        out_shape=jax.ShapeDtypeStruct((D, S), A_x.dtype),
        scratch_shapes=[
            pltpu.VMEM((ng, 128, S), _BF16),
            pltpu.VMEM((ng, S, 128), _BF16),
            pltpu.VMEM((ng, 128, S), _BF16),
            pltpu.VMEM((S, _BQ), _F32),
            pltpu.VMEM((S, _BQ), _F32),
            pltpu.VMEM((2 * D, _BQ), _F32),
            pltpu.VMEM((3 * D, D), _BF16),
            pltpu.VMEM((3 * D, D), _BF16),
            pltpu.VMEM((D, 2 * D), _BF16),
            pltpu.VMEM((8, _BQ), _F32),
            pltpu.VMEM((2, 1, S), _F32),
            pltpu.VMEM((D, S), _BF16),
            pltpu.VMEM((2, D, 3 * D), _BF16),
            pltpu.VMEM((2 * D, D), _BF16),
            pltpu.SemaphoreType.DMA((pl.cdiv(D, 128) + S // _BQ + 3,)),
        ],
        compiler_params=pltpu.CompilerParams(
            dimension_semantics=("arbitrary",),
            vmem_limit_bytes=100 * 1024 * 1024,
        ),
    )(A_x.reshape(S, D).T, A_wqkv, A_wo, B_wqkv, B_wo, gate_w)
    return out.T.reshape(B, S, D)
```

```python
import functools
import math

import jax
import jax.numpy as jnp
from jax import lax
import jax.experimental.pallas as pl
import jax.experimental.pallas.tpu as pltpu


_NN = (((1,), (0,)), ((), ()))
_F32 = jnp.float32
_BF16 = jnp.bfloat16

_H = 16
_HP = 32
_BQ = 512
_BK = 128
_UNROLL = 8
_LEAD = 2


def _kernel(x_hbm, wa_hbm, woa_hbm, wb_hbm, wob_hbm, gw_ref, o_ref,
            qt_s, k_s, vt_s, s0, s1, ot_s, wta_s, wtb_s, wo_s, m_s, g_s, x_ref, w_s, wor_s, sems, *, S, D):
    dh = D // _H
    ntile = _H // 4
    nq = S // _BQ
    nch = S // _BK
    NU = 2 * _H
    qscale = (dh ** -0.5) * math.log2(math.e)
    i = pl.program_id(0)

    def getq(u, qb, j):
        cols = pl.ds(pl.multiple_of(qb * _BQ, _BQ), _BQ)
        parts = [jnp.zeros((_HP * j, _BQ), _BF16)] if j > 0 else []
        parts.append(qt_s[u >> 2, _HP * j:_HP * (j + 1), cols])
        if j < 3:
            parts.append(jnp.zeros((128 - _HP * (j + 1), _BQ), _BF16))
        return jnp.concatenate(parts, axis=0)

    def stage_a(u, qm, c, sbuf, mx):
        st = lax.dot_general(k_s[u >> 2, pl.ds(c * _BK, _BK), :], qm, _NN,
                             preferred_element_type=_F32)
        sbuf[pl.ds(c * _BK, _BK), :] = st
        cm = jnp.max(st.reshape(_BK // 8, 8, _BQ), axis=0)
        return cm if mx is None else jnp.maximum(mx, cm)

    def stage_b(u, j, c, sbuf, m, acc):
        p = jnp.exp2(sbuf[pl.ds(c * _BK, _BK), :] - m).astype(_BF16)
        vt = vt_s[u >> 2, _HP * j:_HP * (j + 1), pl.ds(c * _BK, _BK)]
        r = lax.dot_general(vt, p, _NN, preferred_element_type=_F32)
        return r if acc is None else acc + r

    def finish(u, j, acc):
        gate = g_s[u >> 4, :, pl.ds(pl.multiple_of(i * _BQ, _BQ), _BQ)]
        o = acc * (gate / acc[dh:dh + 1, :])
        sh = (dh * j) % 8
        assert sh in (0, 4)
        base = pl.multiple_of(u * dh - sh, 8)
        if sh:
            o = pltpu.roll(o, sh, 0)
            keep = lax.broadcasted_iota(jnp.int32, (8, _BQ), 0) < sh
            head = jnp.where(keep, ot_s[pl.ds(base, 8), :], o[0:8])
            o = jnp.concatenate([head, o[8:]], axis=0)
        ot_s[pl.ds(base, _HP), :] = o

    @pl.when(i == 0)
    def _prologue():
        rparts = [(r, min(r + 128, D)) for r in range(0, D, 128)]
        srcs = [(wa_hbm.at[r0:r1], w_s.at[0, r0:r1]) for r0, r1 in rparts]
        srcs += [(x_hbm.at[:, _BQ * n:_BQ * (n + 1)], x_ref.at[:, _BQ * n:_BQ * (n + 1)]) for n in range(nq)]
        srcs += [(wb_hbm, w_s.at[1]), (woa_hbm, wor_s.at[0:D]), (wob_hbm, wor_s.at[D:2 * D])]
        cps = [pltpu.make_async_copy(src, dst, sems.at[n]) for n, (src, dst) in enumerate(srcs)]
        cp_x, cp_wb, cp_wo = cps[len(rparts):len(rparts) + nq], cps[-3], cps[-2:]
        for cp in cps[:len(rparts) + 1]:
            cp.start()
        for n, (r0, r1) in enumerate(rparts):
            cps[n].wait()
            if n == len(rparts) - 1:
                cp_x[1].start()
                cp_wb.start()
            wta_s[:, r0:r1] = w_s[0, r0:r1, :].T
        cp_x[0].wait()
        WP = 512
        WE = (3 * D) // 128 * 128
        assert nq == 4 and 2 * WP <= WE <= 3 * WP and 2 * D <= 2 * nq * 128

        gw = jnp.broadcast_to(gw_ref[...].reshape(1, D), (16, D))
        prow = lax.broadcasted_iota(jnp.int32, (128, _BQ), 0) & (_HP - 1)

        def heads4(r, rr, t):
            parts = []
            for h in range(4 * t, 4 * t + 4):
                off = dh * h
                sh = off % 8
                assert sh in (0, 4)
                parts.append(r[off:off + _HP] if sh == 0 else rr[off - 4:off - 4 + _HP])
            return jnp.concatenate(parts, axis=0)

        def proj(c, carry, b):
            if b == 0:
                @pl.when(c == 1)
                def _():
                    cp_x[1].wait()
                    cp_wb.wait()
                    cp_x[2].start()
                    cp_x[3].start()

                @pl.when(c == 2)
                def _():
                    cp_x[2].wait()
                    for cp in cp_wo:
                        cp.start()

                @pl.when(c == 3)
                def _():
                    cp_x[3].wait()

                p0 = pl.multiple_of(jnp.clip((c - 1) * WP, 0, WE - WP), 128)
                bsrc = jnp.minimum(c, 1)
                wtb_s[pl.ds(p0, WP), :] = w_s[bsrc, :, pl.ds(p0, WP)].T
                wtb_s[WE:3 * D, :] = w_s[bsrc, :, WE:3 * D].T
            else:
                for tt in range(2):
                    r0 = pl.multiple_of(jnp.minimum(2 * c + tt, 2 * D // 128 - 1) * 128, 128)
                    wo_s[:, pl.ds(r0, 128)] = wor_s[pl.ds(r0, 128), :].T
            c0 = pl.multiple_of(c * _BQ, _BQ)
            cols = pl.ds(c0, _BQ)
            xt = x_ref[:, cols]
            for part in range(3):
                lhs = (wta_s, wtb_s)[b][part * D:(part + 1) * D, :]
                with_gate = b == 0 and part == 0
                if with_gate:
                    lhs = jnp.concatenate([lhs, gw], axis=0)
                r = lax.dot_general(lhs, xt, _NN, preferred_element_type=_F32)
                if with_gate:
                    g = jax.nn.sigmoid(r[D:D + 1])
                    g_s[0, :, cols] = g
                    g_s[1, :, cols] = 1.0 - g
                    r = r[:D]
                rr = pltpu.roll(r, D - 4, 0)
                for t in range(ntile):
                    y = heads4(r, rr, t)
                    gi = b * ntile + t
                    if part == 0:
                        qt_s[gi, :, cols] = jnp.where(prow < dh, y * qscale, 0.0).astype(_BF16)
                    elif part == 1:
                        k_s[gi, cols, :] = jnp.where(prow < dh, y, 0.0).astype(_BF16).T
                    else:
                        y = jnp.where(prow < dh, y, jnp.where(prow == dh, 1.0, 0.0))
                        vt_s[gi, :, cols] = y.astype(_BF16)
            return carry

        lax.fori_loop(0, nq, functools.partial(proj, b=0), 0)
        for cp in cp_wo:
            cp.wait()
        lax.fori_loop(0, nq, functools.partial(proj, b=1), 0, unroll=2)

        qm = getq(0, 0, 0)
        mx = None
        for c in range(nch):
            mx = stage_a(0, qm, c, s0, mx)
        m_s[...] = mx

    def step(u, j, m, sb, sa, skip_a):
        un = u + 1
        last = un == NU
        qb = jnp.where(last, jnp.minimum(i + 1, nq - 1), i)
        un = jnp.where(last, 0, un)
        qm = getq(un, qb, (j + 1) % 4)
        m = jnp.broadcast_to(jnp.max(m, axis=0, keepdims=True), (8, _BQ))
        always = jnp.broadcast_to(g_s[0, :, 0:_BQ], (8, _BQ)) > -1.0
        mx, acc, toks = None, None, {}
        for n in range(nch + _LEAD):
            if n < nch and not skip_a:
                mx = stage_a(un, qm, n, sa, mx)
                toks[n] = mx
            c = n - _LEAD
            if c >= 0:
                tok = toks.get(c - 1) if c % 2 == 0 else None
                mm = m if tok is None else jnp.where(always, m, tok)
                acc = stage_b(u, j, c, sb, mm[0:1, :], acc)
        finish(u, j, acc)
        return m if skip_a else mx

    def region(t, final):
        m = m_s[...]
        for r in range(_UNROLL):
            j = r % 4
            sb, sa = (s0, s1) if j % 2 == 0 else (s1, s0)
            m = step(_UNROLL * t + r, j, m, sb, sa, skip_a=final and r == _UNROLL - 1)
        m_s[...] = m

    def body(t, carry):
        fin = jnp.logical_and(i == nq - 1, t == NU // _UNROLL - 1)
        pl.when(jnp.logical_not(fin))(functools.partial(region, t, False))
        pl.when(fin)(functools.partial(region, t, True))
        return carry

    lax.fori_loop(0, NU // _UNROLL, body, 0)

    out = lax.dot_general(wo_s[...], ot_s[...].astype(_BF16), _NN, preferred_element_type=_F32)
    o_ref[...] = out.astype(o_ref.dtype)


@jax.jit
def pallas_gated_mix__mha_block__softmax_full_mha__prompt_kernel(
    A_x: jax.Array,
    A_wqkv: jax.Array,
    A_wo: jax.Array,
    B_x: jax.Array,
    B_wqkv: jax.Array,
    B_wo: jax.Array,
    gate_w: jax.Array,
):
    del B_x
    B, S, D = A_x.shape
    assert B == 1 and D % _H == 0 and D // _H < _HP and S == 4 * _BQ and (2 * D) % 128 == 0
    ng = 2 * _H // 4

    def full(shape):
        return pl.BlockSpec(shape, lambda i: (0,) * len(shape))

    out = pl.pallas_call(
        functools.partial(_kernel, S=S, D=D),
        grid=(S // _BQ,),
        in_specs=[pl.BlockSpec(memory_space=pl.ANY)] * 5 + [full((D,))],
        out_specs=pl.BlockSpec((D, _BQ), lambda i: (0, i)),
        out_shape=jax.ShapeDtypeStruct((D, S), A_x.dtype),
        scratch_shapes=[
            pltpu.VMEM((ng, 128, S), _BF16),
            pltpu.VMEM((ng, S, 128), _BF16),
            pltpu.VMEM((ng, 128, S), _BF16),
            pltpu.VMEM((S, _BQ), _F32),
            pltpu.VMEM((S, _BQ), _F32),
            pltpu.VMEM((2 * D, _BQ), _F32),
            pltpu.VMEM((3 * D, D), _BF16),
            pltpu.VMEM((3 * D, D), _BF16),
            pltpu.VMEM((D, 2 * D), _BF16),
            pltpu.VMEM((8, _BQ), _F32),
            pltpu.VMEM((2, 1, S), _F32),
            pltpu.VMEM((D, S), _BF16),
            pltpu.VMEM((2, D, 3 * D), _BF16),
            pltpu.VMEM((2 * D, D), _BF16),
            pltpu.SemaphoreType.DMA((pl.cdiv(D, 128) + S // _BQ + 3,)),
        ],
        compiler_params=pltpu.CompilerParams(
            dimension_semantics=("arbitrary",),
            vmem_limit_bytes=100 * 1024 * 1024,
        ),
    )(A_x.reshape(S, D).T, A_wqkv, A_wo, B_wqkv, B_wo, gate_w)
    return out.T.reshape(B, S, D)
```
